```python
import jax
import jax.numpy as jnp

def _softmax(x, axis=-1):
    return jax.nn.softmax(x, axis=axis)
def _gelu(x):
    return jax.nn.gelu(x, approximate=True)
def _silu(x):
    return jax.nn.silu(x)
def _sigmoid(x):
    return jax.nn.sigmoid(x)
def _layernorm(x, axis=-1, eps=1e-5):
    m = jnp.mean(x, axis=axis, keepdims=True)
    v = jnp.var(x, axis=axis, keepdims=True)
    return (x - m) / jnp.sqrt(v + eps)
def _scatter_add(tgt, idx, src, axis=0):
    return tgt.at[idx].add(src)
def _segment_sum(src, seg, n):
    return jax.ops.segment_sum(src, seg, n)
class _Rng:
    def __init__(self, key):
        self._k = key
    def _next(self):
        self._k, sub = jax.random.split(self._k)
        return sub
    def normal(self, shape):
        return jax.random.normal(self._next(), shape, dtype=jnp.bfloat16)
    def randint(self, lo, hi, shape):
        return jax.random.randint(self._next(), shape, lo, hi, dtype=jnp.int32)
    def uniform(self, shape, lo=0.0, hi=1.0):
        return jax.random.uniform(self._next(), shape, jnp.bfloat16, lo, hi)
    def permutation(self, n):
        return jax.random.permutation(self._next(), n)


kernel_name = 'gated_mix__compressed_kv_cla__ssm_conv_h3__prompt'

def setup_inputs():
    _rng = _Rng(jax.random.key(int.from_bytes(__import__("os").urandom(4), "little")))
    _w = (lambda a: (lambda t: t.astype(jnp.bfloat16) if jnp.issubdtype(t.dtype, jnp.floating) else t)(jnp.asarray(a)))
    def _A_setup():
        B, H, Sq, Sk, D, M = 1, 32, 2048, 2048, 128, 1024
        Dc = 4 * D
        return {
            "x": _w((lambda *s: _rng.normal(s) * 0.05)(B, Sq, M)),
            "c_kv": _w((lambda *s: _rng.normal(s) * 0.05)(B, Sk, Dc)),
            "w_q": _w((lambda *s: _rng.normal(s) * 0.05)(M, H, D) * (M ** -0.5)),
            "w_uk": _w((lambda *s: _rng.normal(s) * 0.05)(Dc, H, D) * (Dc ** -0.5)),
            "w_uv": _w((lambda *s: _rng.normal(s) * 0.05)(Dc, H, D) * (Dc ** -0.5)),
            "w_o": _w((lambda *s: _rng.normal(s) * 0.05)(H, D, M) * ((H * D) ** -0.5)),
        }
    _A_in = _A_setup()

    def _B_setup():
        B, S, D = 1, 2048, 1024
        ks = 4
        return {
            "q": _w((lambda *s: _rng.normal(s) * 0.05)(B, S, D)),
            "k": _w((lambda *s: _rng.normal(s) * 0.05)(B, S, D)),
            "v": _w((lambda *s: _rng.normal(s) * 0.05)(B, S, D)),
            "shift_k": _w((lambda *s: _rng.normal(s) * 0.05)(D, ks) * 0.5),
            "ssm_k": _w((lambda *s: _rng.normal(s) * 0.05)(D, S) * (1.0 / S ** 0.5)),
            "ssm_D": _w((lambda *s: _rng.normal(s) * 0.05)(D)),
        }
    _B_in = _B_setup()

    return {
        "A_x": _A_in["x"],
        "A_c_kv": _A_in["c_kv"],
        "A_w_q": _A_in["w_q"],
        "A_w_uk": _A_in["w_uk"],
        "A_w_uv": _A_in["w_uv"],
        "A_w_o": _A_in["w_o"],
        "B_q": _B_in["q"],
        "B_k": _B_in["k"],
        "B_v": _B_in["v"],
        "B_shift_k": _B_in["shift_k"],
        "B_ssm_k": _B_in["ssm_k"],
        "B_ssm_D": _B_in["ssm_D"],
        "gate_w": _w((lambda *s: _rng.normal(s) * 0.05)(1024)),
    }

def reference(A_x, A_c_kv, A_w_q, A_w_uk, A_w_uv, A_w_o, B_q, B_k, B_v, B_shift_k, B_ssm_k, B_ssm_D, gate_w):
    def _A_ref(x, c_kv, w_q, w_uk, w_uv, w_o):
        B, Sq, M = x.shape[0], x.shape[1], x.shape[2]
        Sk = c_kv.shape[1]
        H, D = w_q.shape[1], w_q.shape[2]
        q = jnp.einsum("bqm,mhd->bhqd", x, w_q)
        k = jnp.einsum("bkc,chd->bhkd", c_kv, w_uk)
        v = jnp.einsum("bkc,chd->bhkd", c_kv, w_uv)
        scores = jnp.einsum("bhqd,bhkd->bhqk", q, k) * (D ** -0.5)
        off = Sk - Sq
        qi = jnp.arange(Sq)[:, None]
        kj = jnp.arange(Sk)[None, :]
        cmask = kj <= (qi + off)
        scores = jnp.where(cmask[None, None], scores, -1e9)
        p = _softmax(scores, axis=-1)
        ctx = jnp.einsum("bhqk,bhkd->bhqd", p, v)
        return jnp.einsum("bhqd,hdm->bqm", ctx, w_o)

    def _B_ref(q, k, v, shift_k, ssm_k, ssm_D):
        B, S, D = q.shape
        ks = shift_k.shape[-1]
        k_pad = jnp.pad(k, ((0, 0), (ks - 1, 0), (0, 0)))
        k_shift = jnp.zeros_like(k)
        for t in range(ks):
            k_shift = k_shift + k_pad[:, t:t + S, :] * shift_k[:, ks - 1 - t][None, None, :]
        kv = k_shift * v
        L = 2 * S
        kv_pad = jnp.pad(kv, ((0, 0), (0, S), (0, 0)))
        kf_pad = jnp.pad(ssm_k, ((0, 0), (0, S)))
        kv_f = (lambda x, axes=(-2,-1): jnp.fft.rfft2(x.astype(jnp.float32), axes=axes))(kv_pad[:, None, :, :], axes=(1, 2))
        kf_f = (lambda x, axes=(-2,-1): jnp.fft.rfft2(x.astype(jnp.float32), axes=axes))(kf_pad[:, None, :], axes=(1, 2))
        kf_f = (lambda x, *d: x.transpose(*d))(kf_f, 1, 2, 0)
        y_f = kv_f * kf_f[None, :, :, :]
        y = (lambda x, s, axes=(-2,-1): jnp.fft.irfft2(x, s=s, axes=axes).astype(jnp.bfloat16))(y_f, (1, L), axes=(1, 2))[:, 0, :S, :]
        y = y + kv * ssm_D[None, None, :]
        return q * y

    x = A_x
    g = _sigmoid((x * gate_w).sum(-1, keepdims=True))
    a = _A_ref(x, A_c_kv, A_w_q, A_w_uk, A_w_uv, A_w_o)
    b = _B_ref(x, B_k, B_v, B_shift_k, B_ssm_k, B_ssm_D)
    return g * a + (1 - g) * b
```

```python
import numpy as np
import jax
import jax.numpy as jnp
from jax import lax
import jax.experimental.pallas as pl
import jax.experimental.pallas.tpu as pltpu

S, M, H, D, DC = 2048, 1024, 32, 128, 512
HG = 4
NG = H // HG
C = 128
NC = S // C
BQ = 256
F32, BF16 = jnp.float32, jnp.bfloat16


def _dft_consts():
    f = np.arange(C)[:, None].astype(np.float64)
    t = np.arange(C)[None, :].astype(np.float64)
    ang = np.pi * (2 * f + 1) * t / (2 * C)
    fwd = np.concatenate([np.cos(ang), -np.sin(ang)], 0)
    inv = np.concatenate([np.cos(ang).T, -np.sin(ang).T], 1) / C
    return fwd.astype(np.float32), inv.astype(np.float32)


_FWD, _INV = _dft_consts()
_NT = (((1,), (1,)), ((), ()))


def _kernel(x_ref, c_ref, wq_ref, wk_ref, wv_ref, wo_ref, xs_ref, bk_ref, bv_ref, sh_ref, h_ref,
            sd_ref, gw_ref, fwd_ref, inv_ref, o_ref,
            acc, g_s, q_s, k_s, v_s, ctx_s, kv_s, hr, hi, xr, xi):
    step = pl.program_id(0)

    @pl.when(step == 0)
    def _():
        acc[...] = jnp.zeros_like(acc)
        z = jnp.sum(x_ref[...].astype(F32) * gw_ref[...].astype(F32), axis=1, keepdims=True)
        g_s[...] = jnp.broadcast_to(1.0 / (1.0 + jnp.exp(-z)), (S, 128))

    q = jnp.dot(x_ref[...], wq_ref[...], preferred_element_type=F32) * (D ** -0.5 * np.log2(np.e))
    q_s[...] = q.astype(BF16)
    k_s[...] = jnp.dot(c_ref[...], wk_ref[...], preferred_element_type=F32).astype(BF16)
    v_s[...] = jnp.dot(c_ref[...], wv_ref[...], preferred_element_type=F32).astype(BF16)

    kk = bk_ref[...].astype(F32)
    sh = sh_ref[...].astype(F32)
    row = lax.broadcasted_iota(jnp.int32, (S, 128), 0)
    ks = kk * sh[0:1]
    for t in range(1, 4):
        ks = ks + jnp.where(row >= t, pltpu.roll(kk, t, 0), 0.0) * sh[t:t + 1]
    kv_s[...] = ks * bv_ref[...].astype(F32)
    fwd = fwd_ref[...]
    fr = lax.broadcasted_iota(jnp.int32, (C, 128), 0)
    sgn = jnp.where(fr % 2 == 0, 1.0, -1.0)
    pr = pi = None
    for j in range(NC):
        xf = jnp.dot(fwd, kv_s[j * C:(j + 1) * C].astype(BF16), preferred_element_type=F32)
        xr[j] = xf[:C]
        xi[j] = xf[C:]
        hf = lax.dot_general(fwd, h_ref[:, j * C:(j + 1) * C], _NT, preferred_element_type=F32)
        a, b = hf[:C], hf[C:]
        if j == 0:
            hr[j] = a
            hi[j] = b
        else:
            hr[j] = a - sgn * pi
            hi[j] = b + sgn * pr
        pr, pi = a, b

    def ssm_chunk(i):
        zr = zi = None
        for j in range(i + 1):
            a, b, c, d = hr[i - j], hi[i - j], xr[j], xi[j]
            tr, ti = a * c - b * d, a * d + b * c
            zr = tr if zr is None else zr + tr
            zi = ti if zi is None else zi + ti
        z = jnp.concatenate([zr, zi], 0).astype(BF16)
        y = jnp.dot(inv_ref[...], z, preferred_element_type=F32)
        r = slice(i * C, (i + 1) * C)
        y = y + kv_s[r] * sd_ref[...].astype(F32)
        col = pl.ds(pl.multiple_of(step * 128, 128), 128)
        acc[r, col] += (1.0 - g_s[r]) * xs_ref[r].astype(F32) * y

    ri = lax.broadcasted_iota(jnp.int32, (BQ, BQ), 0)
    ci = lax.broadcasted_iota(jnp.int32, (BQ, BQ), 1)
    tri = ci <= ri
    nq = S // BQ
    n = 0
    for hh in range(HG):
        hs = slice(hh * D, (hh + 1) * D)
        for qi in range(nq):
            r = slice(qi * BQ, (qi + 1) * BQ)
            e = (qi + 1) * BQ
            qb = q_s[r, hs]
            sd = lax.dot_general(qb, k_s[r, hs], _NT, preferred_element_type=F32)
            sd = jnp.where(tri, sd, -1e30)
            m = jnp.max(sd, axis=1, keepdims=True)
            if qi > 0:
                so = lax.dot_general(qb, k_s[0:qi * BQ, hs], _NT, preferred_element_type=F32)
                m = jnp.maximum(m, jnp.max(so, axis=1, keepdims=True))
            p = jnp.exp2(sd - m)
            l = jnp.sum(p, axis=1, keepdims=True)
            o = jnp.dot(p.astype(BF16), v_s[r, hs], preferred_element_type=F32)
            if qi > 0:
                po = jnp.exp2(so - m)
                l = l + jnp.sum(po, axis=1, keepdims=True)
                o = o + jnp.dot(po.astype(BF16), v_s[0:qi * BQ, hs], preferred_element_type=F32)
            ctx_s[r, hs] = (o * (g_s[r] / l)).astype(BF16)
            if n % 2 == 0:
                ssm_chunk(n // 2)
            n += 1

    acc[...] += jnp.dot(ctx_s[...], wo_ref[...], preferred_element_type=F32)

    @pl.when(step == NG - 1)
    def _():
        o_ref[...] = acc[...].astype(o_ref.dtype)


@jax.jit
def pallas_gated_mix__compressed_kv_cla__ssm_conv_h3__prompt_kernel(
    A_x, A_c_kv, A_w_q, A_w_uk, A_w_uv, A_w_o, B_q, B_k, B_v, B_shift_k, B_ssm_k, B_ssm_D, gate_w,
):
    x = A_x.reshape(S, M)
    one = pl.Buffered(1)
    full = lambda shp: pl.BlockSpec(shp, lambda i: (0, 0), pipeline_mode=one)
    colb = lambda r: pl.BlockSpec((r, 128), lambda i: (0, i))
    V = pltpu.VMEM
    out = pl.pallas_call(
        _kernel,
        grid=(NG,),
        in_specs=[
            full((S, M)), full((S, DC)),
            pl.BlockSpec((M, HG * D), lambda i: (0, i)),
            pl.BlockSpec((DC, HG * D), lambda i: (0, i)),
            pl.BlockSpec((DC, HG * D), lambda i: (0, i)),
            pl.BlockSpec((HG * D, M), lambda i: (i, 0)),
            colb(S), colb(S), colb(S), colb(4),
            pl.BlockSpec((128, S), lambda i: (i, 0)),
            colb(1), full((1, M)), full((2 * C, C)), full((C, 2 * C)),
        ],
        out_specs=pl.BlockSpec((S, M), lambda i: (0, 0)),
        out_shape=jax.ShapeDtypeStruct((S, M), BF16),
        scratch_shapes=[
            V((S, M), F32), V((S, 128), F32),
            V((S, HG * D), BF16), V((S, HG * D), BF16), V((S, HG * D), BF16), V((S, HG * D), BF16),
            V((S, 128), F32),
            V((NC, C, 128), F32), V((NC, C, 128), F32), V((NC, C, 128), F32), V((NC, C, 128), F32),
        ],
        compiler_params=pltpu.CompilerParams(
            dimension_semantics=("arbitrary",), vmem_limit_bytes=110 * 1024 * 1024),
    )(x, A_c_kv.reshape(S, DC), A_w_q.reshape(M, H * D), A_w_uk.reshape(DC, H * D),
      A_w_uv.reshape(DC, H * D), A_w_o.reshape(H * D, M), x, B_k.reshape(S, M), B_v.reshape(S, M),
      B_shift_k.T, B_ssm_k, B_ssm_D.reshape(1, M), gate_w.reshape(1, M),
      jnp.asarray(_FWD, BF16), jnp.asarray(_INV, BF16))
    return out.reshape(1, S, M)
```

```python
import numpy as np
import jax
import jax.numpy as jnp
from jax import lax
import jax.experimental.pallas as pl
import jax.experimental.pallas.tpu as pltpu

S, M, H, D, DC = 2048, 1024, 32, 128, 512
HG = 4
NG = H // HG
C = 128
NC = S // C
BQ = 256
F32, BF16 = jnp.float32, jnp.bfloat16


def _dft_consts():
    f = np.arange(C)[:, None].astype(np.float64)
    t = np.arange(C)[None, :].astype(np.float64)
    ang = np.pi * (2 * f + 1) * t / (2 * C)
    fwd = np.concatenate([np.cos(ang), -np.sin(ang)], 0)
    inv = np.concatenate([np.cos(ang).T, -np.sin(ang).T], 1) / C
    return fwd.astype(np.float32), inv.astype(np.float32)


_FWD, _INV = _dft_consts()
_NT = (((1,), (1,)), ((), ()))


def _kernel(x_ref, c_ref, wq_ref, wk_ref, wv_ref, wo_ref, xs_ref, bk_ref, bv_ref, sh_ref, h_ref,
            sd_ref, gw_ref, fwd_ref, inv_ref, o_ref,
            acc, g_s, q_s, k_s, v_s, ctx_s, kv_s, hr, hi, xr, xi, z_s):
    step = pl.program_id(0)

    @pl.when(step == 0)
    def _():
        acc[...] = jnp.zeros_like(acc)
        z = jnp.sum(x_ref[...].astype(F32) * gw_ref[...].astype(F32), axis=1, keepdims=True)
        g_s[...] = jnp.broadcast_to(1.0 / (1.0 + jnp.exp(-z)), (S, 128))

    def kvproj(i):
        r = slice(i * 512, (i + 1) * 512)
        k_s[r] = jnp.dot(c_ref[r], wk_ref[...], preferred_element_type=F32).astype(BF16)
        v_s[r] = jnp.dot(c_ref[r], wv_ref[...], preferred_element_type=F32).astype(BF16)

    def qproj(i):
        r = slice(i * 512, (i + 1) * 512)
        q = jnp.dot(x_ref[r], wq_ref[...], preferred_element_type=F32)
        q_s[r] = (q * (D ** -0.5 * np.log2(np.e))).astype(BF16)

    kk = bk_ref[...].astype(F32)
    sh = sh_ref[...].astype(F32)
    row = lax.broadcasted_iota(jnp.int32, (S, 128), 0)
    ks = kk * sh[0:1]
    for t in range(1, 4):
        ks = ks + jnp.where(row >= t, pltpu.roll(kk, t, 0), 0.0) * sh[t:t + 1]
    kv_s[...] = ks * bv_ref[...].astype(F32)
    fwd = fwd_ref[...]
    fr = lax.broadcasted_iota(jnp.int32, (C, 128), 0)
    sgn = jnp.where(fr % 2 == 0, 1.0, -1.0)
    pr = pi = None
    for j in range(NC):
        if j % 4 == 0:
            kvproj(j // 4)
        if j % 4 == 2:
            qproj(j // 4)
        xf = jnp.dot(fwd, kv_s[j * C:(j + 1) * C].astype(BF16), preferred_element_type=F32)
        xr[j] = xf[:C]
        xi[j] = xf[C:]
        hf = lax.dot_general(fwd, h_ref[:, j * C:(j + 1) * C], _NT, preferred_element_type=F32)
        a, b = hf[:C], hf[C:]
        if j == 0:
            hr[j] = a
            hi[j] = b
        else:
            hr[j] = a - sgn * pi
            hi[j] = b + sgn * pr
        pr, pi = a, b

    def ssm_mac(i, hh):
        fs = pl.ds(pl.multiple_of(hh * 32, 32), 32)
        zr = zi = None
        for j in range(i + 1):
            a, b, c, d = hr[i - j, fs], hi[i - j, fs], xr[j, fs], xi[j, fs]
            tr, ti = a * c - b * d, a * d + b * c
            zr = tr if zr is None else zr + tr
            zi = ti if zi is None else zi + ti
        z_s[i, fs] = zr.astype(BF16)
        z_s[i, pl.ds(pl.multiple_of(C + hh * 32, 32), 32)] = zi.astype(BF16)

    def ssm_out(i):
        y = jnp.dot(inv_ref[...], z_s[i], preferred_element_type=F32)
        r = slice(i * C, (i + 1) * C)
        y = y + kv_s[r] * sd_ref[...].astype(F32)
        col = pl.ds(pl.multiple_of(step * 128, 128), 128)
        acc[r, col] += (1.0 - g_s[r]) * xs_ref[r].astype(F32) * y

    ri = lax.broadcasted_iota(jnp.int32, (BQ, BQ), 0)
    ci = lax.broadcasted_iota(jnp.int32, (BQ, BQ), 1)
    tri = ci <= ri
    nq = S // BQ

    @pl.loop(0, HG)
    def _(hh):
        hs = pl.ds(pl.multiple_of(hh * D, D), D)
        for qi in range(nq):
            r = slice(qi * BQ, (qi + 1) * BQ)
            e = (qi + 1) * BQ
            qb = q_s[r, hs]
            sd = lax.dot_general(qb, k_s[r, hs], _NT, preferred_element_type=F32)
            sd = jnp.where(tri, sd, -1e30)
            m = jnp.max(sd, axis=1, keepdims=True)
            if qi > 0:
                so = lax.dot_general(qb, k_s[0:qi * BQ, hs], _NT, preferred_element_type=F32)
                m = jnp.maximum(m, jnp.max(so, axis=1, keepdims=True))
            p = jnp.exp2(sd - m)
            l = jnp.sum(p, axis=1, keepdims=True)
            o = jnp.dot(p.astype(BF16), v_s[r, hs], preferred_element_type=F32)
            if qi > 0:
                po = jnp.exp2(so - m)
                l = l + jnp.sum(po, axis=1, keepdims=True)
                o = o + jnp.dot(po.astype(BF16), v_s[0:qi * BQ, hs], preferred_element_type=F32)
            ctx_s[r, hs] = (o * (g_s[r] / l)).astype(BF16)
            ssm_mac(2 * qi, hh)
            ssm_mac(2 * qi + 1, hh)

    for qi in range(nq):
        r = slice(qi * BQ, (qi + 1) * BQ)
        ssm_out(2 * qi)
        ssm_out(2 * qi + 1)
        acc[r] += jnp.dot(ctx_s[r], wo_ref[...], preferred_element_type=F32)

    @pl.when(step == NG - 1)
    def _():
        o_ref[...] = acc[...].astype(o_ref.dtype)


@jax.jit
def pallas_gated_mix__compressed_kv_cla__ssm_conv_h3__prompt_kernel(
    A_x, A_c_kv, A_w_q, A_w_uk, A_w_uv, A_w_o, B_q, B_k, B_v, B_shift_k, B_ssm_k, B_ssm_D, gate_w,
):
    x = A_x.reshape(S, M)
    one = pl.Buffered(1)
    full = lambda shp: pl.BlockSpec(shp, lambda i: (0, 0), pipeline_mode=one)
    colb = lambda r: pl.BlockSpec((r, 128), lambda i: (0, i))
    V = pltpu.VMEM
    out = pl.pallas_call(
        _kernel,
        grid=(NG,),
        in_specs=[
            full((S, M)), full((S, DC)),
            pl.BlockSpec((M, HG * D), lambda i: (0, i)),
            pl.BlockSpec((DC, HG * D), lambda i: (0, i)),
            pl.BlockSpec((DC, HG * D), lambda i: (0, i)),
            pl.BlockSpec((HG * D, M), lambda i: (i, 0)),
            colb(S), colb(S), colb(S), colb(4),
            pl.BlockSpec((128, S), lambda i: (i, 0)),
            colb(1), full((1, M)), full((2 * C, C)), full((C, 2 * C)),
        ],
        out_specs=pl.BlockSpec((S, M), lambda i: (0, 0)),
        out_shape=jax.ShapeDtypeStruct((S, M), BF16),
        scratch_shapes=[
            V((S, M), F32), V((S, 128), F32),
            V((S, HG * D), BF16), V((S, HG * D), BF16), V((S, HG * D), BF16), V((S, HG * D), BF16),
            V((S, 128), F32),
            V((NC, C, 128), F32), V((NC, C, 128), F32), V((NC, C, 128), F32), V((NC, C, 128), F32),
            V((NC, 2 * C, 128), BF16),
        ],
        compiler_params=pltpu.CompilerParams(
            dimension_semantics=("arbitrary",), vmem_limit_bytes=110 * 1024 * 1024),
    )(x, A_c_kv.reshape(S, DC), A_w_q.reshape(M, H * D), A_w_uk.reshape(DC, H * D),
      A_w_uv.reshape(DC, H * D), A_w_o.reshape(H * D, M), x, B_k.reshape(S, M), B_v.reshape(S, M),
      B_shift_k.T, B_ssm_k, B_ssm_D.reshape(1, M), gate_w.reshape(1, M),
      jnp.asarray(_FWD, BF16), jnp.asarray(_INV, BF16))
    return out.reshape(1, S, M)
```

```python
import numpy as np
import jax
import jax.numpy as jnp
from jax import lax
import jax.experimental.pallas as pl
import jax.experimental.pallas.tpu as pltpu

S, M, H, D, DC = 2048, 1024, 32, 128, 512
HG = 4
NG = H // HG
C = 128
NC = S // C
BQ = 256
F32, BF16 = jnp.float32, jnp.bfloat16


def _dft_consts():
    f = np.arange(C)[:, None].astype(np.float64)
    t = np.arange(C)[None, :].astype(np.float64)
    ang = np.pi * (2 * f + 1) * t / (2 * C)
    fwd = np.concatenate([np.cos(ang), -np.sin(ang)], 0)
    inv = np.concatenate([np.cos(ang).T, -np.sin(ang).T], 1) / C
    return fwd.astype(np.float32), inv.astype(np.float32)


_FWD, _INV = _dft_consts()
_NT = (((1,), (1,)), ((), ()))


def _kernel(x_ref, c_ref, wq_ref, wk_ref, wv_ref, wo_ref, xs_ref, bk_ref, bv_ref, sh_ref, h_ref,
            sd_ref, gw_ref, fwd_ref, inv_ref, o_ref,
            acc, g_s, q_s, k_s, v_s, ctx_s, kv_s, hr, hi, xr, xi, z_s, prev):
    step = pl.program_id(0)

    @pl.when(step == 0)
    def _():
        acc[...] = jnp.zeros_like(acc)
        z = jnp.sum(x_ref[...].astype(F32) * gw_ref[...].astype(F32), axis=1, keepdims=True)
        g_s[...] = jnp.broadcast_to(1.0 / (1.0 + jnp.exp(-z)), (S, 128))

    def kvproj(i):
        r = pl.ds(pl.multiple_of(i * 512, 512), 512)
        k_s[r] = jnp.dot(c_ref[r], wk_ref[...], preferred_element_type=F32).astype(BF16)
        v_s[r] = jnp.dot(c_ref[r], wv_ref[...], preferred_element_type=F32).astype(BF16)

    def qproj(i):
        r = pl.ds(pl.multiple_of(i * 512, 512), 512)
        q = jnp.dot(x_ref[r], wq_ref[...], preferred_element_type=F32)
        q_s[r] = (q * (D ** -0.5 * np.log2(np.e))).astype(BF16)

    kk = bk_ref[...].astype(F32)
    sh = sh_ref[...].astype(F32)
    row = lax.broadcasted_iota(jnp.int32, (S, 128), 0)
    ks = kk * sh[0:1]
    for t in range(1, 4):
        ks = ks + jnp.where(row >= t, pltpu.roll(kk, t, 0), 0.0) * sh[t:t + 1]
    kv_s[...] = ks * bv_ref[...].astype(F32)
    fwd = fwd_ref[...]
    fr = lax.broadcasted_iota(jnp.int32, (C, 128), 0)
    sgn = jnp.where(fr % 2 == 0, 1.0, -1.0)
    prev[...] = jnp.zeros_like(prev)

    @pl.loop(0, S // 512)
    def _(ib):
        kvproj(ib)
        qproj(ib)
        pr, pi = prev[:C], prev[C:]
        for jj in range(4):
            j = ib * 4 + jj
            ts = pl.ds(pl.multiple_of(j * C, C), C)
            xf = jnp.dot(fwd, kv_s[ts].astype(BF16), preferred_element_type=F32)
            xr[j] = xf[:C]
            xi[j] = xf[C:]
            hf = lax.dot_general(fwd, h_ref[:, ts], _NT, preferred_element_type=F32)
            a, b = hf[:C], hf[C:]
            hr[j] = a - sgn * pi
            hi[j] = b + sgn * pr
            pr, pi = a, b
        prev[:C] = pr
        prev[C:] = pi

    def ssm_mac(i, hh):
        fs = pl.ds(pl.multiple_of(hh * 32, 32), 32)
        zr = zi = None
        for j in range(i + 1):
            a, b, c, d = hr[i - j, fs], hi[i - j, fs], xr[j, fs], xi[j, fs]
            tr, ti = a * c - b * d, a * d + b * c
            zr = tr if zr is None else zr + tr
            zi = ti if zi is None else zi + ti
        z_s[i, fs] = zr.astype(BF16)
        z_s[i, pl.ds(pl.multiple_of(C + hh * 32, 32), 32)] = zi.astype(BF16)

    def ssm_out(i):
        y = jnp.dot(inv_ref[...], z_s[i], preferred_element_type=F32)
        r = pl.ds(pl.multiple_of(i * C, C), C)
        y = y + kv_s[r] * sd_ref[...].astype(F32)
        col = pl.ds(pl.multiple_of(step * 128, 128), 128)
        acc[r, col] += (1.0 - g_s[r]) * xs_ref[r].astype(F32) * y

    ri = lax.broadcasted_iota(jnp.int32, (BQ, BQ), 0)
    ci = lax.broadcasted_iota(jnp.int32, (BQ, BQ), 1)
    tri = ci <= ri
    nq = S // BQ

    @pl.loop(0, HG)
    def _(hh):
        hs = pl.ds(pl.multiple_of(hh * D, D), D)
        for qi in range(nq):
            r = slice(qi * BQ, (qi + 1) * BQ)
            e = (qi + 1) * BQ
            qb = q_s[r, hs]
            sd = lax.dot_general(qb, k_s[r, hs], _NT, preferred_element_type=F32)
            sd = jnp.where(tri, sd, -1e30)
            m = jnp.max(sd, axis=1, keepdims=True)
            if qi > 0:
                so = lax.dot_general(qb, k_s[0:qi * BQ, hs], _NT, preferred_element_type=F32)
                m = jnp.maximum(m, jnp.max(so, axis=1, keepdims=True))
            p = jnp.exp2(sd - m)
            l = jnp.sum(p, axis=1, keepdims=True)
            o = jnp.dot(p.astype(BF16), v_s[r, hs], preferred_element_type=F32)
            if qi > 0:
                po = jnp.exp2(so - m)
                l = l + jnp.sum(po, axis=1, keepdims=True)
                o = o + jnp.dot(po.astype(BF16), v_s[0:qi * BQ, hs], preferred_element_type=F32)
            ctx_s[r, hs] = (o * (g_s[r] / l)).astype(BF16)
            ssm_mac(2 * qi, hh)
            ssm_mac(2 * qi + 1, hh)

    @pl.loop(0, S // 512)
    def _(ib):
        r = pl.ds(pl.multiple_of(ib * 512, 512), 512)
        for jj in range(4):
            ssm_out(ib * 4 + jj)
        acc[r] += jnp.dot(ctx_s[r], wo_ref[...], preferred_element_type=F32)

        @pl.when(step == NG - 1)
        def _():
            o_ref[r] = acc[r].astype(o_ref.dtype)


@jax.jit
def pallas_gated_mix__compressed_kv_cla__ssm_conv_h3__prompt_kernel(
    A_x, A_c_kv, A_w_q, A_w_uk, A_w_uv, A_w_o, B_q, B_k, B_v, B_shift_k, B_ssm_k, B_ssm_D, gate_w,
):
    x = A_x.reshape(S, M)
    one = pl.Buffered(1)
    full = lambda shp: pl.BlockSpec(shp, lambda i: (0, 0), pipeline_mode=one)
    colb = lambda r: pl.BlockSpec((r, 128), lambda i: (0, i))
    V = pltpu.VMEM
    out = pl.pallas_call(
        _kernel,
        grid=(NG,),
        in_specs=[
            full((S, M)), full((S, DC)),
            pl.BlockSpec((M, HG * D), lambda i: (0, i)),
            pl.BlockSpec((DC, HG * D), lambda i: (0, i)),
            pl.BlockSpec((DC, HG * D), lambda i: (0, i)),
            pl.BlockSpec((HG * D, M), lambda i: (i, 0)),
            colb(S), colb(S), colb(S), colb(4),
            pl.BlockSpec((128, S), lambda i: (i, 0)),
            colb(1), full((1, M)), full((2 * C, C)), full((C, 2 * C)),
        ],
        out_specs=pl.BlockSpec((S, M), lambda i: (0, 0)),
        out_shape=jax.ShapeDtypeStruct((S, M), BF16),
        scratch_shapes=[
            V((S, M), F32), V((S, 128), F32),
            V((S, HG * D), BF16), V((S, HG * D), BF16), V((S, HG * D), BF16), V((S, HG * D), BF16),
            V((S, 128), F32),
            V((NC, C, 128), F32), V((NC, C, 128), F32), V((NC, C, 128), F32), V((NC, C, 128), F32),
            V((NC, 2 * C, 128), BF16), V((2 * C, 128), F32),
        ],
        compiler_params=pltpu.CompilerParams(
            dimension_semantics=("arbitrary",), vmem_limit_bytes=110 * 1024 * 1024),
    )(x, A_c_kv.reshape(S, DC), A_w_q.reshape(M, H * D), A_w_uk.reshape(DC, H * D),
      A_w_uv.reshape(DC, H * D), A_w_o.reshape(H * D, M), x, B_k.reshape(S, M), B_v.reshape(S, M),
      B_shift_k.T, B_ssm_k, B_ssm_D.reshape(1, M), gate_w.reshape(1, M),
      jnp.asarray(_FWD, BF16), jnp.asarray(_INV, BF16))
    return out.reshape(1, S, M)
```

```python
import numpy as np
import jax
import jax.numpy as jnp
from jax import lax
import jax.experimental.pallas as pl
import jax.experimental.pallas.tpu as pltpu

S, M, H, D, DC = 2048, 1024, 32, 128, 512
HG = 4
NG = H // HG
C = 128
NC = S // C
BQ = 256
F32, BF16 = jnp.float32, jnp.bfloat16


def _dft_consts():
    f = np.arange(C)[:, None].astype(np.float64)
    t = np.arange(C)[None, :].astype(np.float64)
    ang = np.pi * (2 * f + 1) * t / (2 * C)
    fwd = np.concatenate([np.cos(ang), -np.sin(ang)], 0)
    inv = np.concatenate([np.cos(ang).T, -np.sin(ang).T], 1) / C
    return fwd.astype(np.float32), inv.astype(np.float32)


_FWD, _INV = _dft_consts()
_NT = (((1,), (1,)), ((), ()))


def _kernel(x_ref, c_ref, wq_ref, wk_ref, wv_ref, wo_ref, xs_ref, bk_ref, bv_ref, sh_ref, h_ref,
            sd_ref, gw_ref, fwd_ref, inv_ref, o_ref,
            acc, g_s, q_s, k_s, v_s, ctx_s, kv_s, hr, hi, xr, xi, z_s, prev, qm, km):
    step = pl.program_id(0)

    @pl.when(step == 0)
    def _():
        acc[...] = jnp.zeros_like(acc)
        z = jnp.sum(x_ref[...].astype(F32) * gw_ref[...].astype(F32), axis=1, keepdims=True)
        g_s[...] = jnp.broadcast_to(1.0 / (1.0 + jnp.exp(-z)), (S, 128))

    def kvproj(i):
        r = pl.ds(pl.multiple_of(i * 512, 512), 512)
        kf = jnp.dot(c_ref[r], wk_ref[...], preferred_element_type=F32)
        k_s[r] = kf.astype(BF16)
        km[...] = jnp.maximum(km[...], jnp.max(jnp.abs(kf).reshape(64, 8, HG * D), axis=0))
        v_s[r] = jnp.dot(c_ref[r], wv_ref[...], preferred_element_type=F32).astype(BF16)

    def qproj(i):
        r = pl.ds(pl.multiple_of(i * 512, 512), 512)
        q = jnp.dot(x_ref[r], wq_ref[...], preferred_element_type=F32)
        q = q * (D ** -0.5 * np.log2(np.e))
        q_s[r] = q.astype(BF16)
        qm[...] = jnp.maximum(qm[...], jnp.max(jnp.abs(q).reshape(64, 8, HG * D), axis=0))

    kk = bk_ref[...].astype(F32)
    sh = sh_ref[...].astype(F32)
    row = lax.broadcasted_iota(jnp.int32, (S, 128), 0)
    ks = kk * sh[0:1]
    for t in range(1, 4):
        ks = ks + jnp.where(row >= t, pltpu.roll(kk, t, 0), 0.0) * sh[t:t + 1]
    kv_s[...] = ks * bv_ref[...].astype(F32)
    fwd = fwd_ref[...]
    fr = lax.broadcasted_iota(jnp.int32, (C, 128), 0)
    sgn = jnp.where(fr % 2 == 0, 1.0, -1.0)
    prev[...] = jnp.zeros_like(prev)
    qm[...] = jnp.zeros_like(qm)
    km[...] = jnp.zeros_like(km)

    @pl.loop(0, S // 512)
    def _(ib):
        kvproj(ib)
        qproj(ib)
        pr, pi = prev[:C], prev[C:]
        for jj in range(4):
            j = ib * 4 + jj
            ts = pl.ds(pl.multiple_of(j * C, C), C)
            xf = jnp.dot(fwd, kv_s[ts].astype(BF16), preferred_element_type=F32)
            xr[j] = xf[:C]
            xi[j] = xf[C:]
            hf = lax.dot_general(fwd, h_ref[:, ts], _NT, preferred_element_type=F32)
            a, b = hf[:C], hf[C:]
            hr[j] = a - sgn * pi
            hi[j] = b + sgn * pr
            pr, pi = a, b
        prev[:C] = pr
        prev[C:] = pi

    def ssm_mac(i, hh):
        fs = pl.ds(pl.multiple_of(hh * 32, 32), 32)
        zr = zi = None
        for j in range(i + 1):
            a, b, c, d = hr[i - j, fs], hi[i - j, fs], xr[j, fs], xi[j, fs]
            tr, ti = a * c - b * d, a * d + b * c
            zr = tr if zr is None else zr + tr
            zi = ti if zi is None else zi + ti
        z_s[i, fs] = zr.astype(BF16)
        z_s[i, pl.ds(pl.multiple_of(C + hh * 32, 32), 32)] = zi.astype(BF16)

    def ssm_out(i):
        y = jnp.dot(inv_ref[...], z_s[i], preferred_element_type=F32)
        r = pl.ds(pl.multiple_of(i * C, C), C)
        y = y + kv_s[r] * sd_ref[...].astype(F32)
        col = pl.ds(pl.multiple_of(step * 128, 128), 128)
        acc[r, col] += (1.0 - g_s[r]) * xs_ref[r].astype(F32) * y

    ri = lax.broadcasted_iota(jnp.int32, (BQ, BQ), 0)
    ci = lax.broadcasted_iota(jnp.int32, (BQ, BQ), 1)
    tri = ci <= ri
    nq = S // BQ

    def attend(hh, guard):
        hs = pl.ds(pl.multiple_of(hh * D, D), D)
        for qi in range(nq):
            r = slice(qi * BQ, (qi + 1) * BQ)
            qb = q_s[r, hs]
            sd = lax.dot_general(qb, k_s[r, hs], _NT, preferred_element_type=F32)
            if qi > 0:
                so = lax.dot_general(qb, k_s[0:qi * BQ, hs], _NT, preferred_element_type=F32)
            if guard:
                sd = jnp.where(tri, sd, -1e30)
                m = jnp.max(sd, axis=1, keepdims=True)
                if qi > 0:
                    m = jnp.maximum(m, jnp.max(so, axis=1, keepdims=True))
                    so = so - m
                p = jnp.exp2(sd - m)
            else:
                p = jnp.where(tri, jnp.exp2(sd), 0.0)
            l = jnp.sum(p, axis=1, keepdims=True)
            o = jnp.dot(p.astype(BF16), v_s[r, hs], preferred_element_type=F32)
            if qi > 0:
                po = jnp.exp2(so)
                l = l + jnp.sum(po, axis=1, keepdims=True)
                o = o + jnp.dot(po.astype(BF16), v_s[0:qi * BQ, hs], preferred_element_type=F32)
            ctx_s[r, hs] = (o * (g_s[r] / l)).astype(BF16)
            ssm_mac(2 * qi, hh)
            ssm_mac(2 * qi + 1, hh)

    prod = jnp.max(qm[...], axis=0, keepdims=True) * jnp.max(km[...], axis=0, keepdims=True)
    bound = prod[:, 0:D]
    for hh in range(1, HG):
        bound = jnp.maximum(bound, prod[:, hh * D:(hh + 1) * D])
    safe = jnp.sum(bound) <= 50.0

    @pl.when(safe)
    def _():
        pl.loop(0, HG)(lambda hh: attend(hh, False))

    @pl.when(jnp.logical_not(safe))
    def _():
        pl.loop(0, HG)(lambda hh: attend(hh, True))

    @pl.loop(0, S // 512)
    def _(ib):
        r = pl.ds(pl.multiple_of(ib * 512, 512), 512)
        for jj in range(4):
            ssm_out(ib * 4 + jj)
        acc[r] += jnp.dot(ctx_s[r], wo_ref[...], preferred_element_type=F32)

        @pl.when(step == NG - 1)
        def _():
            o_ref[r] = acc[r].astype(o_ref.dtype)


@jax.jit
def pallas_gated_mix__compressed_kv_cla__ssm_conv_h3__prompt_kernel(
    A_x, A_c_kv, A_w_q, A_w_uk, A_w_uv, A_w_o, B_q, B_k, B_v, B_shift_k, B_ssm_k, B_ssm_D, gate_w,
):
    x = A_x.reshape(S, M)
    one = pl.Buffered(1)
    full = lambda shp: pl.BlockSpec(shp, lambda i: (0, 0), pipeline_mode=one)
    colb = lambda r: pl.BlockSpec((r, 128), lambda i: (0, i))
    V = pltpu.VMEM
    out = pl.pallas_call(
        _kernel,
        grid=(NG,),
        in_specs=[
            full((S, M)), full((S, DC)),
            pl.BlockSpec((M, HG * D), lambda i: (0, i)),
            pl.BlockSpec((DC, HG * D), lambda i: (0, i)),
            pl.BlockSpec((DC, HG * D), lambda i: (0, i)),
            pl.BlockSpec((HG * D, M), lambda i: (i, 0)),
            colb(S), colb(S), colb(S), colb(4),
            pl.BlockSpec((128, S), lambda i: (i, 0)),
            colb(1), full((1, M)), full((2 * C, C)), full((C, 2 * C)),
        ],
        out_specs=pl.BlockSpec((S, M), lambda i: (0, 0)),
        out_shape=jax.ShapeDtypeStruct((S, M), BF16),
        scratch_shapes=[
            V((S, M), F32), V((S, 128), F32),
            V((S, HG * D), BF16), V((S, HG * D), BF16), V((S, HG * D), BF16), V((S, HG * D), BF16),
            V((S, 128), F32),
            V((NC, C, 128), F32), V((NC, C, 128), F32), V((NC, C, 128), F32), V((NC, C, 128), F32),
            V((NC, 2 * C, 128), BF16), V((2 * C, 128), F32),
            V((8, HG * D), F32), V((8, HG * D), F32),
        ],
        compiler_params=pltpu.CompilerParams(
            dimension_semantics=("arbitrary",), vmem_limit_bytes=110 * 1024 * 1024),
    )(x, A_c_kv.reshape(S, DC), A_w_q.reshape(M, H * D), A_w_uk.reshape(DC, H * D),
      A_w_uv.reshape(DC, H * D), A_w_o.reshape(H * D, M), x, B_k.reshape(S, M), B_v.reshape(S, M),
      B_shift_k.T, B_ssm_k, B_ssm_D.reshape(1, M), gate_w.reshape(1, M),
      jnp.asarray(_FWD, BF16), jnp.asarray(_INV, BF16))
    return out.reshape(1, S, M)
```

```python
import numpy as np
import jax
import jax.numpy as jnp
from jax import lax
import jax.experimental.pallas as pl
import jax.experimental.pallas.tpu as pltpu

S, M, H, D, DC = 2048, 1024, 32, 128, 512
HG = 4
NG = H // HG
C = 128
NC = S // C
BQ = 256
FQ = 512
KC = 256
F32, BF16 = jnp.float32, jnp.bfloat16


def _dft_consts():
    f = np.arange(C)[:, None].astype(np.float64)
    t = np.arange(C)[None, :].astype(np.float64)
    ang = np.pi * (2 * f + 1) * t / (2 * C)
    fwd = np.concatenate([np.cos(ang), -np.sin(ang)], 0)
    inv = np.concatenate([np.cos(ang).T, -np.sin(ang).T], 1) / C
    return fwd.astype(np.float32), inv.astype(np.float32)


_FWD, _INV = _dft_consts()
_NT = (((1,), (1,)), ((), ()))


def _kernel(x_ref, c_ref, wq_ref, wk_ref, wv_ref, wo_ref, xs_ref, bk_ref, bv_ref, sh_ref, h_ref,
            sd_ref, gw_ref, fwd_ref, inv_ref, o_ref,
            acc, g_s, q_s, k_s, v_s, ctx_s, kv_s, hr, hi, xr, xi, z_s, prev, qm, km):
    step = pl.program_id(0)

    @pl.when(step == 0)
    def _():
        acc[...] = jnp.zeros_like(acc)
        z = jnp.sum(x_ref[...].astype(F32) * gw_ref[...].astype(F32), axis=1, keepdims=True)
        g_s[...] = jnp.broadcast_to(1.0 / (1.0 + jnp.exp(-z)), (S, 128))

    def kvproj(i):
        r = pl.ds(pl.multiple_of(i * 512, 512), 512)
        kf = jnp.dot(c_ref[r], wk_ref[...], preferred_element_type=F32)
        k_s[r] = kf.astype(BF16)
        km[...] = jnp.maximum(km[...], jnp.max(jnp.abs(kf).reshape(64, 8, HG * D), axis=0))
        v_s[r] = jnp.dot(c_ref[r], wv_ref[...], preferred_element_type=F32).astype(BF16)

    def qproj(i):
        r = pl.ds(pl.multiple_of(i * 512, 512), 512)
        q = jnp.dot(x_ref[r], wq_ref[...], preferred_element_type=F32)
        q = q * (D ** -0.5 * np.log2(np.e))
        q_s[r] = q.astype(BF16)
        qm[...] = jnp.maximum(qm[...], jnp.max(jnp.abs(q).reshape(64, 8, HG * D), axis=0))

    kk = bk_ref[...].astype(F32)
    sh = sh_ref[...].astype(F32)
    row = lax.broadcasted_iota(jnp.int32, (S, 128), 0)
    ks = kk * sh[0:1]
    for t in range(1, 4):
        ks = ks + jnp.where(row >= t, pltpu.roll(kk, t, 0), 0.0) * sh[t:t + 1]
    kv_s[...] = ks * bv_ref[...].astype(F32)
    fwd = fwd_ref[...]
    fr = lax.broadcasted_iota(jnp.int32, (C, 128), 0)
    sgn = jnp.where(fr % 2 == 0, 1.0, -1.0)
    prev[...] = jnp.zeros_like(prev)
    qm[...] = jnp.zeros_like(qm)
    km[...] = jnp.zeros_like(km)

    @pl.loop(0, S // 512)
    def _(ib):
        kvproj(ib)
        qproj(ib)
        pr, pi = prev[:C], prev[C:]
        for jj in range(4):
            j = ib * 4 + jj
            ts = pl.ds(pl.multiple_of(j * C, C), C)
            xf = jnp.dot(fwd, kv_s[ts].astype(BF16), preferred_element_type=F32)
            xr[j] = xf[:C]
            xi[j] = xf[C:]
            hf = lax.dot_general(fwd, h_ref[:, ts], _NT, preferred_element_type=F32)
            a, b = hf[:C], hf[C:]
            hr[j] = a - sgn * pi
            hi[j] = b + sgn * pr
            pr, pi = a, b
        prev[:C] = pr
        prev[C:] = pi

    def ssm_mac(i, hh):
        fs = pl.ds(pl.multiple_of(hh * 32, 32), 32)
        zr = zi = None
        for j in range(i + 1):
            a, b, c, d = hr[i - j, fs], hi[i - j, fs], xr[j, fs], xi[j, fs]
            tr, ti = a * c - b * d, a * d + b * c
            zr = tr if zr is None else zr + tr
            zi = ti if zi is None else zi + ti
        z_s[i, fs] = zr.astype(BF16)
        z_s[i, pl.ds(pl.multiple_of(C + hh * 32, 32), 32)] = zi.astype(BF16)

    def ssm_out(i):
        y = jnp.dot(inv_ref[...], z_s[i], preferred_element_type=F32)
        r = pl.ds(pl.multiple_of(i * C, C), C)
        y = y + kv_s[r] * sd_ref[...].astype(F32)
        col = pl.ds(pl.multiple_of(step * 128, 128), 128)
        acc[r, col] += (1.0 - g_s[r]) * xs_ref[r].astype(F32) * y

    ri = lax.broadcasted_iota(jnp.int32, (BQ, BQ), 0)
    ci = lax.broadcasted_iota(jnp.int32, (BQ, BQ), 1)
    tri = ci <= ri
    nq = S // BQ

    def attend(hh, guard):
        hs = pl.ds(pl.multiple_of(hh * D, D), D)
        for qi in range(nq):
            r = slice(qi * BQ, (qi + 1) * BQ)
            qb = q_s[r, hs]
            sd = lax.dot_general(qb, k_s[r, hs], _NT, preferred_element_type=F32)
            if qi > 0:
                so = lax.dot_general(qb, k_s[0:qi * BQ, hs], _NT, preferred_element_type=F32)
            if guard:
                sd = jnp.where(tri, sd, -1e30)
                m = jnp.max(sd, axis=1, keepdims=True)
                if qi > 0:
                    m = jnp.maximum(m, jnp.max(so, axis=1, keepdims=True))
                    so = so - m
                p = jnp.exp2(sd - m)
            else:
                p = jnp.where(tri, jnp.exp2(sd), 0.0)
            l = jnp.sum(p, axis=1, keepdims=True)
            o = jnp.dot(p.astype(BF16), v_s[r, hs], preferred_element_type=F32)
            if qi > 0:
                po = jnp.exp2(so)
                l = l + jnp.sum(po, axis=1, keepdims=True)
                o = o + jnp.dot(po.astype(BF16), v_s[0:qi * BQ, hs], preferred_element_type=F32)
            ctx_s[r, hs] = (o * (g_s[r] / l)).astype(BF16)
            ssm_mac(2 * qi, hh)
            ssm_mac(2 * qi + 1, hh)

    def attend_fast(hh):
        hs = pl.ds(pl.multiple_of(hh * D, D), D)
        t128 = tri[:128, :128]
        for q0 in range(0, S, FQ):
            o = l = None
            for k0 in [*range(0, q0, KC), *range(q0, q0 + FQ, 128)]:
                kw = min(KC, q0 - k0) if k0 < q0 else 128
                r0 = max(q0, k0)
                rs = slice(r0, q0 + FQ)
                ks_ = slice(k0, k0 + kw)
                p = jnp.exp2(lax.dot_general(q_s[rs, hs], k_s[ks_, hs], _NT,
                                             preferred_element_type=F32))
                if k0 >= q0:
                    top = jnp.where(t128, p[:128], 0.0)
                    p = top if p.shape[0] == 128 else jnp.concatenate([top, p[128:]], 0)
                pv = jnp.dot(p.astype(BF16), v_s[ks_, hs], preferred_element_type=F32)
                p = sum(p[:, c:c + 128] for c in range(0, kw, 128))
                if o is None:
                    o, l = pv, p
                elif r0 == q0:
                    o, l = o + pv, l + p
                else:
                    n = r0 - q0
                    o = jnp.concatenate([o[:n], o[n:] + pv], 0)
                    l = jnp.concatenate([l[:n], l[n:] + p], 0)
            r = slice(q0, q0 + FQ)
            ctx_s[r, hs] = (o * (g_s[r] / jnp.sum(l, axis=1, keepdims=True))).astype(BF16)
            for i in range(q0 // C, (q0 + FQ) // C):
                ssm_mac(i, hh)

    prod = jnp.max(qm[...], axis=0, keepdims=True) * jnp.max(km[...], axis=0, keepdims=True)
    bound = prod[:, 0:D]
    for hh in range(1, HG):
        bound = jnp.maximum(bound, prod[:, hh * D:(hh + 1) * D])
    safe = jnp.sum(bound) <= 50.0

    @pl.when(safe)
    def _():
        pl.loop(0, HG)(attend_fast)

    @pl.when(jnp.logical_not(safe))
    def _():
        pl.loop(0, HG)(lambda hh: attend(hh, True))

    @pl.loop(0, S // 512)
    def _(ib):
        r = pl.ds(pl.multiple_of(ib * 512, 512), 512)
        for jj in range(4):
            ssm_out(ib * 4 + jj)
        acc[r] += jnp.dot(ctx_s[r], wo_ref[...], preferred_element_type=F32)

        @pl.when(step == NG - 1)
        def _():
            o_ref[r] = acc[r].astype(o_ref.dtype)


@jax.jit
def pallas_gated_mix__compressed_kv_cla__ssm_conv_h3__prompt_kernel(
    A_x, A_c_kv, A_w_q, A_w_uk, A_w_uv, A_w_o, B_q, B_k, B_v, B_shift_k, B_ssm_k, B_ssm_D, gate_w,
):
    x = A_x.reshape(S, M)
    one = pl.Buffered(1)
    full = lambda shp: pl.BlockSpec(shp, lambda i: (0, 0), pipeline_mode=one)
    colb = lambda r: pl.BlockSpec((r, 128), lambda i: (0, i))
    V = pltpu.VMEM
    out = pl.pallas_call(
        _kernel,
        grid=(NG,),
        in_specs=[
            full((S, M)), full((S, DC)),
            pl.BlockSpec((M, HG * D), lambda i: (0, i)),
            pl.BlockSpec((DC, HG * D), lambda i: (0, i)),
            pl.BlockSpec((DC, HG * D), lambda i: (0, i)),
            pl.BlockSpec((HG * D, M), lambda i: (i, 0)),
            colb(S), colb(S), colb(S), colb(4),
            pl.BlockSpec((128, S), lambda i: (i, 0)),
            colb(1), full((1, M)), full((2 * C, C)), full((C, 2 * C)),
        ],
        out_specs=pl.BlockSpec((S, M), lambda i: (0, 0)),
        out_shape=jax.ShapeDtypeStruct((S, M), BF16),
        scratch_shapes=[
            V((S, M), F32), V((S, 128), F32),
            V((S, HG * D), BF16), V((S, HG * D), BF16), V((S, HG * D), BF16), V((S, HG * D), BF16),
            V((S, 128), F32),
            V((NC, C, 128), F32), V((NC, C, 128), F32), V((NC, C, 128), F32), V((NC, C, 128), F32),
            V((NC, 2 * C, 128), BF16), V((2 * C, 128), F32),
            V((8, HG * D), F32), V((8, HG * D), F32),
        ],
        compiler_params=pltpu.CompilerParams(
            dimension_semantics=("arbitrary",), vmem_limit_bytes=110 * 1024 * 1024),
    )(x, A_c_kv.reshape(S, DC), A_w_q.reshape(M, H * D), A_w_uk.reshape(DC, H * D),
      A_w_uv.reshape(DC, H * D), A_w_o.reshape(H * D, M), x, B_k.reshape(S, M), B_v.reshape(S, M),
      B_shift_k.T, B_ssm_k, B_ssm_D.reshape(1, M), gate_w.reshape(1, M),
      jnp.asarray(_FWD, BF16), jnp.asarray(_INV, BF16))
    return out.reshape(1, S, M)
```
